```python
import jax
import jax.numpy as jnp

def _softmax(x, axis=-1):
    return jax.nn.softmax(x, axis=axis)
def _gelu(x):
    return jax.nn.gelu(x, approximate=True)
def _silu(x):
    return jax.nn.silu(x)
def _sigmoid(x):
    return jax.nn.sigmoid(x)
def _layernorm(x, axis=-1, eps=1e-5):
    m = jnp.mean(x, axis=axis, keepdims=True)
    v = jnp.var(x, axis=axis, keepdims=True)
    return (x - m) / jnp.sqrt(v + eps)
def _scatter_add(tgt, idx, src, axis=0):
    return tgt.at[idx].add(src)
def _segment_sum(src, seg, n):
    return jax.ops.segment_sum(src, seg, n)
class _Rng:
    def __init__(self, key):
        self._k = key
    def _next(self):
        self._k, sub = jax.random.split(self._k)
        return sub
    def normal(self, shape):
        return jax.random.normal(self._next(), shape, dtype=jnp.bfloat16)
    def randint(self, lo, hi, shape):
        return jax.random.randint(self._next(), shape, lo, hi, dtype=jnp.int32)
    def uniform(self, shape, lo=0.0, hi=1.0):
        return jax.random.uniform(self._next(), shape, jnp.bfloat16, lo, hi)
    def permutation(self, n):
        return jax.random.permutation(self._next(), n)


kernel_name = 'standalone__winograd__vision'

def setup_inputs():
    _rng = _Rng(jax.random.key(int.from_bytes(__import__("os").urandom(4), "little")))
    _w = (lambda a: (lambda t: t.astype(jnp.bfloat16) if jnp.issubdtype(t.dtype, jnp.floating) else t)(jnp.asarray(a)))
    H = W = 512 // 2 * 2
    C = 192
    return {
        "x": _w((lambda *s: _rng.normal(s) * 0.05)(1, H, W, C)),
        "w": _w((lambda *s: _rng.normal(s) * 0.05)(3, 3, C, C)),
    }

def reference(x, w):
    N, H, W, C = x.shape
    K = w.shape[-1]
    G  = jnp.array([[1.0,0.0,0.0],[0.5,0.5,0.5],[0.5,-0.5,0.5],[0.0,0.0,1.0]], dtype=x.dtype)
    Bt = jnp.array([[1.0,0.0,-1.0,0.0],[0.0,1.0,1.0,0.0],[0.0,-1.0,1.0,0.0],[0.0,1.0,0.0,-1.0]], dtype=x.dtype)
    At = jnp.array([[1.0,1.0,1.0,0.0],[0.0,1.0,-1.0,-1.0]], dtype=x.dtype)
    U = jnp.einsum("ar,rsck,bs->abck", G, w, G)
    xp = jnp.pad(x, ((0,0),(1,1),(1,1),(0,0)))
    nH, nW = H // 2, W // 2
    patches = []
    for i in range(4):
        for j in range(4):
            patches.append(xp[:, i:i + 2 * nH:2, j:j + 2 * nW:2, :])
    d = jnp.stack(patches).reshape(4, 4, N * nH * nW, C)
    V = jnp.einsum("ai,ijpc,bj->abpc", Bt, d, Bt)
    M = jnp.einsum("abck,abpc->abpk", U, V)
    Y = jnp.einsum("ma,abpk,nb->pmnk", At, M, At)
    Y = Y.reshape(N, nH, nW, 2, 2, K)
    Y = (lambda x, *d: x.transpose(*d))(Y, 0, 1, 3, 2, 4, 5).reshape(N, H, W, K)
    return Y
```

```python
import functools
import jax, jax.numpy as jnp, numpy as np
import jax.experimental.pallas as pl
import jax.experimental.pallas.tpu as pltpu

def mats(m,pts):
    n=m+2; a=[float(p) for p in pts]
    AT=np.array([[p**i for p in a]+[1.0 if i==m-1 else 0.0] for i in range(m)])
    f=[np.prod([a[i]-a[j] for j in range(n-1) if j!=i]) for i in range(n-1)]
    G=np.array([[a[i]**j/f[i] for j in range(3)] for i in range(n-1)]+[[0,0,1.0]])
    BT=[]
    for i in range(n-1):
        p=np.array([1.0])
        for j in range(n-1):
            if j!=i: p=np.convolve(p,[-a[j],1.0])
        BT.append(np.concatenate([p,[0.0]]))
    p=np.array([1.0])
    for j in range(n-1): p=np.convolve(p,[-a[j],1.0])
    BT.append(p)
    return AT,G,np.array(BT)

def lincomb(coefs, vals):
    acc=None
    for c,v in zip(coefs,vals):
        c=float(c)
        if c==0: continue
        if acc is None:
            acc = v() if c==1 else (-v() if c==-1 else c*v())
        else:
            acc = acc+v() if c==1 else (acc-v() if c==-1 else acc+c*v())
    return acc

def make(m, pts, TH):
    AT,G,BT=mats(m,pts); n=m+2
    C=192; W=512; H=512
    def kern(xm_ref, xt_ref, xb_ref, w_ref, o_ref, u_ref, v_ref):
        i=pl.program_id(0)
        @pl.when(i==0)
        def _():
            for a in range(n):
                for s in range(3):
                    u=lincomb(G[a],[lambda r=r: w_ref[r,s].astype(jnp.float32) for r in range(3)])
                    u_ref[a,:,s*C:(s+1)*C]=u.T.astype(jnp.bfloat16)
        nb=pl.num_programs(0)
        def row(r):
            if r<0:
                return jnp.where(i>0, xt_ref[0].astype(jnp.float32), 0.0)
            if r>=TH:
                return jnp.where(i<nb-1, xb_ref[0].astype(jnp.float32), 0.0)
            return xm_ref[r].astype(jnp.float32)
        lane=jax.lax.broadcasted_iota(jnp.int32,(C//2,W),1)
        for t in range(TH//m):
            for a in range(n):
                v=lincomb(BT[a],[lambda j=j: row(t*m-1+j) for j in range(n)]).astype(jnp.bfloat16)
                vi=pltpu.bitcast(v,jnp.uint32)
                l=jnp.where(lane==0,jnp.uint32(0),pltpu.roll(vi,1,1))
                r=jnp.where(lane==W-1,jnp.uint32(0),pltpu.roll(vi,W-1,1))
                v_ref[a,0:C]=pltpu.bitcast(l,jnp.bfloat16)
                v_ref[a,C:2*C]=v
                v_ref[a,2*C:3*C]=pltpu.bitcast(r,jnp.bfloat16)
            M=[jnp.dot(u_ref[a],v_ref[a],preferred_element_type=jnp.float32) for a in range(n)]
            for q in range(m):
                o_ref[t*m+q]=lincomb(AT[q],[lambda a=a: M[a] for a in range(n)]).astype(jnp.bfloat16)
    @jax.jit
    def f(x,w):
        xt=jnp.transpose(x[0],(0,2,1))
        out=pl.pallas_call(kern,grid=(H//TH,),
            in_specs=[pl.BlockSpec((TH,C,W),lambda i:(i,0,0)),
                      pl.BlockSpec((1,C,W),lambda i:(jnp.maximum(i*TH-1,0),0,0)),
                      pl.BlockSpec((1,C,W),lambda i:(jnp.minimum((i+1)*TH,H-1),0,0)),
                      pl.BlockSpec((3,3,C,C),lambda i:(0,0,0,0))],
            out_specs=pl.BlockSpec((TH,C,W),lambda i:(i,0,0)),
            out_shape=jax.ShapeDtypeStruct((H,C,W),jnp.bfloat16),
            scratch_shapes=[pltpu.VMEM((n,C,3*C),jnp.bfloat16),pltpu.VMEM((n,3*C,W),jnp.bfloat16)],
            compiler_params=pltpu.CompilerParams(dimension_semantics=("arbitrary",),vmem_limit_bytes=100*1024*1024),
        )(xt,xt,xt,w)
        return jnp.transpose(out,(0,2,1))[None]
    return f
_impl = make(4, [0, 1, -1, .5, -2], 16)

@jax.jit
def pallas_standalone__winograd__vision_kernel(x: jax.Array, w: jax.Array):
    return _impl(x, w)
```
